```python
import os as _os
_os.environ.setdefault("JAX_PLATFORMS", "cpu")
import jax
import jax.numpy as jnp

def _softmax(x, axis=-1):
    return jax.nn.softmax(x, axis=axis)
def _gelu(x):
    return jax.nn.gelu(x, approximate=True)
def _silu(x):
    return jax.nn.silu(x)
def _sigmoid(x):
    return jax.nn.sigmoid(x)
def _layernorm(x, axis=-1, eps=1e-5):
    m = jnp.mean(x, axis=axis, keepdims=True)
    v = jnp.var(x, axis=axis, keepdims=True)
    return (x - m) / jnp.sqrt(v + eps)
def _scatter_add(tgt, idx, src, axis=0):
    return tgt.at[idx].add(src)
def _segment_sum(src, seg, n):
    return jax.ops.segment_sum(src, seg, n)
class _Rng:
    def __init__(self, key):
        self._k = key
    def _next(self):
        self._k, sub = jax.random.split(self._k)
        return sub
    def normal(self, shape):
        return jax.random.normal(self._next(), shape, dtype=jnp.bfloat16)
    def randint(self, lo, hi, shape):
        return jax.random.randint(self._next(), shape, lo, hi, dtype=jnp.int32)
    def uniform(self, shape, lo=0.0, hi=1.0):
        return jax.random.uniform(self._next(), shape, jnp.bfloat16, lo, hi)
    def permutation(self, n):
        return jax.random.permutation(self._next(), n)


kernel_name = 'interleave_layers__linear_attn_block__mha_block__prompt'

def setup_inputs():
    _rng = _Rng(jax.random.key(int.from_bytes(__import__("os").urandom(4), "little")))
    _w = (lambda a: (lambda t: t.astype(jnp.bfloat16) if jnp.issubdtype(t.dtype, jnp.floating) else t)(jnp.asarray(a)))
    def _A_setup():
        B, S, D = 1, 2048, 640
        return {
            "x": _w((lambda *s: _rng.normal(s) * 0.05)(B, S, D)),
            "wqkv": _w((lambda *s: _rng.normal(s) * 0.1)(D, 3 * D)),
            "wo": _w((lambda *s: _rng.normal(s) * 0.05)(D, D)),
        }
    _A_in = _A_setup()

    def _B_setup():
        B, S, D, H = 1, 2048, 640, 32
        return {
            "x": _w((lambda *s: _rng.normal(s) * 0.05)(B, S, D)),
            "wqkv": _w((lambda *s: _rng.normal(s) * 0.1)(D, 3 * D)),
            "wo": _w((lambda *s: _rng.normal(s) * 0.05)(D, D)),
        }
    _B_in = _B_setup()

    return {
        "A_x": _A_in["x"],
        "A_wqkv": _A_in["wqkv"],
        "A_wo": _A_in["wo"],
        "B_x": _B_in["x"],
        "B_wqkv": _B_in["wqkv"],
        "B_wo": _B_in["wo"],
    }

def reference(A_x, A_wqkv, A_wo, B_x, B_wqkv, B_wo):
    def _A_ref(x, wqkv, wo):
        B, S, D = x.shape
        H = 32; Dh = D // H
        qkv = (lambda x, *d: x.transpose(*d))((x @ wqkv).reshape(B, S, 3, H, Dh), 2, 0, 3, 1, 4)
        q, k, v = qkv[0], qkv[1], qkv[2]
        phi = lambda t: jnp.where(t > 0, t + 1, jnp.exp(t)) + 1e-6
        pq, pk = phi(q), phi(k)
        kv = jnp.einsum("bhsd,bhse->bhde", pk, v)
        z = jnp.einsum("bhsd->bhd", pk)
        num = jnp.einsum("bhqd,bhde->bhqe", pq, kv)
        den = jnp.einsum("bhqd,bhd->bhq", pq, z)[..., None] + 1e-6
        o = num / den
        return (lambda x, *d: x.transpose(*d))(o, 0, 2, 1, 3).reshape(B, S, D) @ wo

    def _B_ref(x, wqkv, wo):
        B, S, D = x.shape
        H = 32
        Dh = D // H
        qkv = (lambda x, *d: x.transpose(*d))((x @ wqkv).reshape(B, S, 3, H, Dh), 2, 0, 3, 1, 4)
        q, k, v = qkv[0], qkv[1], qkv[2]
        scores = jnp.einsum("bhqd,bhkd->bhqk", q, k) * (Dh ** -0.5)
        p = _softmax(scores, axis=-1)
        o = jnp.einsum("bhqk,bhkd->bhqd", p, v)
        return (lambda x, *d: x.transpose(*d))(o, 0, 2, 1, 3).reshape(B, S, D) @ wo

    x = A_x
    x = x + _A_ref(_layernorm(x, axis=-1), A_wqkv, A_wo)
    x = x + _B_ref(_layernorm(x, axis=-1), B_wqkv, B_wo)
    x = x + _A_ref(_layernorm(x, axis=-1), A_wqkv, A_wo)
    x = x + _B_ref(_layernorm(x, axis=-1), B_wqkv, B_wo)
    return x
```

```python
import math

import jax
import jax.numpy as jnp
from jax import lax
import jax.experimental.pallas as pl
import jax.experimental.pallas.tpu as pltpu

S = 2048
D = 640
H = 32
DH = D // H
RB = 512
NRB = S // RB
HB = RB // 2
QB = 512
CK = 128
LAG = 2
NG = 6
GW = 6 * DH
QROWS = GW * (NG - 1) + 128

BF = jnp.bfloat16
F32 = jnp.float32
U32 = jnp.uint32

_NN = (((1,), (0,)), ((), ()))
_NT = (((1,), (1,)), ((), ()))
_TN = (((0,), (0,)), ((), ()))


def _dot(a, b, dims=_NN):
    return lax.dot_general(a, b, dims, preferred_element_type=F32)


def _layernorm(x):
    m = jnp.mean(x, axis=-1, keepdims=True)
    xc = x - m
    v = jnp.mean(xc * xc, axis=-1, keepdims=True)
    return xc * lax.rsqrt(v + 1e-5)


def _phi(t):
    return jnp.where(t > 0, t + 1.0, jnp.exp(t)) + 1e-6


def _kernel(x_hbm, aqkv_hbm, awo_hbm, bqkv_hbm, bwo_hbm, o_hbm,
            xb_s, aqkv_s, awo_s, bqkv_s, bwo_s,
            x_s, xn_s, pkt_s, z_s, g_s, m_s, zc_s,
            awkt_s, bwqt_s, bwvt_s, bwk_s,
            k_s, qt_s, vt_s, ot_s, sa_s, sb_s, sem_x, sem_w, sem_o):

    def rows(r):
        return pl.ds(pl.multiple_of(r * RB, RB), RB)

    def half_rows(r, h):
        return pl.ds(pl.multiple_of(r * RB + h * HB, HB), HB)

    def x_copy(r):
        return pltpu.make_async_copy(x_hbm.at[r * RB:(r + 1) * RB], xb_s.at[r * RB:(r + 1) * RB], sem_x.at[r])

    def o_copy(r):
        return pltpu.make_async_copy(xb_s.at[rows(r)], o_hbm.at[rows(r)], sem_o.at[r])

    def a_copy(p):
        cols = slice(p * D, (p + 1) * D)
        return pltpu.make_async_copy(aqkv_hbm.at[:, cols], aqkv_s.at[:, cols], sem_w.at[p])

    awo_copy = pltpu.make_async_copy(awo_hbm, awo_s, sem_w.at[3])
    bqkv_copy = pltpu.make_async_copy(bqkv_hbm, bqkv_s, sem_w.at[4])
    bwo_copy = pltpu.make_async_copy(bwo_hbm, bwo_s, sem_w.at[5])

    a_copy(1).start()
    for r in range(NRB):
        x_copy(r).start()
    qt_s[D:, :] = jnp.zeros((QROWS - D, S), F32)
    a_copy(1).wait()
    awkt_s[...] = aqkv_s[:, D:2 * D].astype(F32).T.astype(BF)
    for r in range(NRB):
        x_copy(r).wait()
    a_copy(2).start()
    awo_copy.start()
    a_copy(0).start()
    bqkv_copy.start()
    bwo_copy.start()

    def first_ln(r, c):
        x = xb_s[rows(r), :].astype(F32)
        x_s[rows(r), :] = x
        xn_s[rows(r), :] = _layernorm(x).astype(BF)
        return c

    lax.fori_loop(0, NRB, first_ln, 0)

    def prep_b_weights():
        bqkv_copy.wait()
        bwo_copy.wait()
        bwqt_s[...] = bqkv_s[:, 0:D].astype(F32).T.astype(BF)
        bwvt_s[...] = bqkv_s[:, 2 * D:3 * D].astype(F32).T.astype(BF)
        wk = bqkv_s[:, D:2 * D].astype(F32)
        for g in range(NG - 1):
            bwk_s[:, g * 128:(g + 1) * 128] = wk[:, g * GW:g * GW + 128].astype(BF)
        last = D - GW * (NG - 1)
        lane = lax.broadcasted_iota(jnp.int32, (D, 128), 1)
        tail = pltpu.roll(wk[:, D - 128:], last, 1)
        bwk_s[:, (NG - 1) * 128:] = jnp.where(lane < last, tail, 0.0).astype(BF)

    def phi_kt(r, h, xn):
        pkt = _phi(_dot(awkt_s[...], xn, _NT))
        pkt_s[:, half_rows(r, h)] = pkt.astype(BF)
        zp = pkt[:, 0:128]
        for t in range(1, HB // 128):
            zp = zp + pkt[:, t * 128:(t + 1) * 128]
        return zp

    def lin_a(r, c):
        z_s[r] = sum(phi_kt(r, h, xn_s[half_rows(r, h), :]) for h in range(2))
        return c

    def lin_g(i, c):
        rt = pl.ds(pl.multiple_of(i * 128, 128), 128)
        g_s[rt, :] = _dot(pkt_s[rt, :], xn_s[...]).astype(BF)
        return c

    def lin_b():
        nt = D // 128
        ri = lax.broadcasted_iota(jnp.int32, (128, 128), 0)
        ci = lax.broadcasted_iota(jnp.int32, (1, 128), 1)
        kvs = []
        for i in range(nt):
            lo, hi = max(i - 1, 0), min(i + 2, nt)
            kv = _dot(g_s[i * 128:(i + 1) * 128, :], aqkv_s[:, 2 * D + lo * 128:2 * D + hi * 128])
            parts = []
            for j in range(lo, hi):
                h0 = ((ci + j * 128) // DH) * DH - i * 128
                parts.append(jnp.where((ri >= h0) & (ri < h0 + DH),
                                       kv[:, (j - lo) * 128:(j - lo + 1) * 128], 0.0))
            kvs.append((lo, hi, jnp.concatenate(parts, axis=1).astype(BF)))
        zp = z_s[0]
        for r in range(1, NRB):
            zp = zp + z_s[r]
        z = jnp.sum(zp, axis=1, keepdims=True)
        rd = lax.broadcasted_iota(jnp.int32, (D, 128), 0)
        hd = lax.broadcasted_iota(jnp.int32, (D, 128), 1) * DH
        zc_s[...] = jnp.where((rd >= hd) & (rd < hd + DH), z, 0.0).astype(BF)
        for i, (lo, hi, kv) in enumerate(kvs):
            m_s[i * 128:(i + 1) * 128, :] = _dot(kv, awo_s[lo * 128:hi * 128, :]).astype(BF)

    def lin_c_mha_a(r, c):
        pqs = [_phi(_dot(xn_s[half_rows(r, h), :], aqkv_s[:, 0:D])).astype(BF) for h in range(2)]
        rcp = [1.0 / (_dot(pq, zc_s[...]) + 1e-6) for pq in pqs]
        lane = lax.broadcasted_iota(jnp.int32, (HB, 128), 1)
        xns = []
        for h in range(2):
            rb = jnp.concatenate(
                [jnp.take_along_axis(rcp[h], (lane + j * 128) // DH, axis=1) for j in range(D // 128)],
                axis=1)
            pqn = (pqs[h].astype(F32) * rb).astype(BF)
            x = x_s[half_rows(r, h), :] + _dot(pqn, m_s[...])
            x_s[half_rows(r, h), :] = x
            xns.append(x)
        for h in range(2):
            xns[h] = _layernorm(xns[h]).astype(BF)
            k = _dot(xns[h], bwk_s[...]).astype(BF)
            packed = pl.ds(pl.multiple_of((r * RB + h * HB) // 2, HB // 2), HB // 2)
            for g in range(NG):
                k_s[g, packed, :] = pltpu.bitcast(k[:, g * 128:(g + 1) * 128], U32)
        xn = jnp.concatenate(xns, axis=0)
        qt_s[0:D, rows(r)] = _dot(bwqt_s[...], xn, _NT) * (DH ** -0.5 * math.log2(math.e))
        vt_s[:, rows(r)] = _dot(bwvt_s[...], xn, _NT)
        return c

    npair = H // 2
    NQ = S // QB
    NC = S // CK
    sbuf = (sa_s, sb_s)

    def load_q(g, off, qb):
        ri = lax.broadcasted_iota(jnp.int32, (128, QB), 0)
        q = qt_s[pl.ds(pl.multiple_of(GW * g, 8), 128), qb * QB:(qb + 1) * QB]
        return jnp.where((ri >= off) & (ri < off + DH), q, 0.0).astype(BF)

    def chunk_a(g, q, c, s_out, m):
        kc = pltpu.bitcast(k_s[g, c * CK // 2:(c + 1) * CK // 2, :], BF)
        s = _dot(kc, q)
        s_out[c * CK:(c + 1) * CK, :] = s
        sm = jnp.max(s.reshape(CK // 8, 8, QB), axis=0)
        return sm if m is None else jnp.maximum(m, sm)

    def chunk_b(r0, one, c, s_in, m, acc):
        keys = slice(c * CK, (c + 1) * CK)
        p = jnp.exp2(s_in[keys, :].reshape(CK // 8, 8, QB) - m[None])
        is_one = lax.broadcasted_iota(jnp.int32, (24, CK), 0) == one
        v = jnp.where(is_one, 1.0, vt_s[pl.ds(pl.multiple_of(r0, 8), 24), keys])
        o = _dot(v, p.reshape(CK, QB))
        return o if acc is None else acc + o

    def fin_max(m):
        return jnp.broadcast_to(jnp.max(m, axis=0, keepdims=True), (8, QB))

    def mha_b():
        q = load_q(0, 0, 0)
        m = None
        for c in range(NC):
            m = chunk_a(0, q, c, sa_s, m)

        def body(j, carry):
            m_first, g, off = carry
            wrap = off + 2 * DH >= GW
            g_n = jnp.where(wrap, g + 1, g)
            off_n = jnp.where(wrap, 0, off + 2 * DH)
            r0 = 2 * DH * j
            nb = NQ * 2
            a_items = [(g, off + DH * (n % 2), n // 2) for n in range(1, nb)] + [(g_n, off_n, 0)]
            a_ops = [(n, c) for n in range(nb) for c in range(NC)]
            b_ops = list(a_ops)
            ms = {0: m_first}
            mrun = {}
            qs = {}
            accs = {}
            outs = {}

            def do_a():
                n, c = a_ops.pop(0)
                ga, offa, qb = a_items[n]
                if c == 0:
                    qs[n] = load_q(ga, offa, qb)
                mrun[n] = chunk_a(ga, qs[n], c, sbuf[(n + 1) % 2], mrun.get(n))
                if c == NC - 1:
                    ms[n + 1] = fin_max(mrun[n])

            def do_b():
                n, c = b_ops.pop(0)
                e = n % 2
                one = DH if e == 0 else 0
                accs[n] = chunk_b(r0 + 16 * e, one, c, sbuf[n % 2], ms[n], accs.get(n))
                if c == NC - 1:
                    outs[n] = accs[n] / accs[n][one:one + 1]
                    if e == 1:
                        o0, o1 = outs[n - 1], outs[n]
                        ri = lax.broadcasted_iota(jnp.int32, (8, QB), 0)
                        mid = jnp.where(ri < 4, o0[16:24], o1[0:8])
                        o = jnp.concatenate([o0[0:16], mid, o1[8:24]], axis=0)
                        qb = n // 2
                        ot_s[pl.ds(pl.multiple_of(r0, 8), 2 * DH), qb * QB:(qb + 1) * QB] = o

            for _ in range(LAG):
                do_a()
            while b_ops:
                if a_ops:
                    do_a()
                do_b()
            return ms[nb], g_n, off_n

        lax.fori_loop(0, npair, body, (fin_max(m), 0, 0))

    def mha_out(r, h):
        ot = ot_s[:, half_rows(r, h)].astype(BF)
        return x_s[half_rows(r, h), :] + _dot(ot, bwo_s[...], _TN)

    def mha_c_lin_a(r, c):
        xs = [mha_out(r, h) for h in range(2)]
        zp = 0.0
        for h in range(2):
            x_s[half_rows(r, h), :] = xs[h]
            xn = _layernorm(xs[h]).astype(BF)
            xn_s[half_rows(r, h), :] = xn
            zp = zp + phi_kt(r, h, xn)
        z_s[r] = zp
        return c

    def mha_c_final(r, c):
        for h in range(2):
            xb_s[half_rows(r, h), :] = mha_out(r, h).astype(BF)
        o_copy(r).start()
        return c

    with jax.named_scope("lin_a"):
        lax.fori_loop(0, NRB, lin_a, 0)

    def layer_pair(i, c):
        with jax.named_scope("lin_g"):
            lax.fori_loop(0, D // 128, lin_g, 0)

        @pl.when(i == 0)
        def _():
            a_copy(2).wait()
            awo_copy.wait()
            a_copy(0).wait()
            prep_b_weights()

        with jax.named_scope("lin_b"):
            lin_b()
        with jax.named_scope("lin_c"):
            lax.fori_loop(0, NRB, lin_c_mha_a, 0)
        with jax.named_scope("mha_b"):
            mha_b()

        with jax.named_scope("mha_c"):
            @pl.when(i == 0)
            def _():
                lax.fori_loop(0, NRB, mha_c_lin_a, 0)

            @pl.when(i == 1)
            def _():
                lax.fori_loop(0, NRB, mha_c_final, 0)

        return c

    lax.fori_loop(0, 2, layer_pair, 0)
    for r in range(NRB):
        o_copy(r).wait()


@jax.jit
def pallas_interleave_layers__linear_attn_block__mha_block__prompt_kernel(
    A_x: jax.Array,
    A_wqkv: jax.Array,
    A_wo: jax.Array,
    B_x: jax.Array,
    B_wqkv: jax.Array,
    B_wo: jax.Array,
):
    del B_x
    scratch = [
        pltpu.VMEM((S, D), BF),
        pltpu.VMEM((D, 3 * D), BF),
        pltpu.VMEM((D, D), BF),
        pltpu.VMEM((D, 3 * D), BF),
        pltpu.VMEM((D, D), BF),
        pltpu.VMEM((S, D), F32),
        pltpu.VMEM((S, D), BF),
        pltpu.VMEM((D, S), BF),
        pltpu.VMEM((NRB, D, 128), F32),
        pltpu.VMEM((D, D), BF),
        pltpu.VMEM((D, D), BF),
        pltpu.VMEM((D, 128), BF),
        pltpu.VMEM((D, D), BF),
        pltpu.VMEM((D, D), BF),
        pltpu.VMEM((D, D), BF),
        pltpu.VMEM((D, NG * 128), BF),
        pltpu.VMEM((NG, S // 2, 128), U32),
        pltpu.VMEM((QROWS, S), F32),
        pltpu.VMEM((D, S), F32),
        pltpu.VMEM((D, S), F32),
        pltpu.VMEM((S, QB), F32),
        pltpu.VMEM((S, QB), F32),
        pltpu.SemaphoreType.DMA((NRB,)),
        pltpu.SemaphoreType.DMA((6,)),
        pltpu.SemaphoreType.DMA((NRB,)),
    ]
    hbm = pl.BlockSpec(memory_space=pl.ANY)
    out = pl.pallas_call(
        _kernel,
        out_shape=jax.ShapeDtypeStruct((S, D), A_x.dtype),
        in_specs=[hbm] * 5,
        out_specs=hbm,
        scratch_shapes=scratch,
        compiler_params=pltpu.CompilerParams(vmem_limit_bytes=110 * 1024 * 1024),
        name="interleaved_attention",
    )(A_x.reshape(S, D), A_wqkv, A_wo, B_wqkv, B_wo)
    return out.reshape(A_x.shape)
```

```python
import math

import jax
import jax.numpy as jnp
from jax import lax
import jax.experimental.pallas as pl
import jax.experimental.pallas.tpu as pltpu

S = 2048
D = 640
H = 32
DH = D // H
RB = 512
NRB = S // RB
HB = RB // 2
FB = RB // 4
QB = RB
NQ = S // QB
CK = FB
NC = S // CK
NG = 6
GW = 6 * DH
QROWS = GW * (NG - 1) + 128
VPU_CHUNKS = (0, 2, 6, 8, 10, 12)
VPU_TILES = 2 * len(VPU_CHUNKS)
VPU_SPREAD = 13
Q_SCALE = DH ** -0.5 * math.log2(math.e)

BF = jnp.bfloat16
F32 = jnp.float32
U32 = jnp.uint32

_NN = (((1,), (0,)), ((), ()))
_NT = (((1,), (1,)), ((), ()))
_TN = (((0,), (0,)), ((), ()))


def _dot(a, b, dims=_NN):
    return lax.dot_general(a, b, dims, preferred_element_type=F32)


def _iota(shape, axis):
    return lax.broadcasted_iota(jnp.int32, shape, axis)


def _layernorm(x):
    m = jnp.mean(x, axis=-1, keepdims=True)
    xc = x - m
    v = jnp.mean(xc * xc, axis=-1, keepdims=True)
    return xc * lax.rsqrt(v + 1e-5)


def _phi(t):
    return jnp.where(t > 0, t + 1.0, jnp.exp(t)) + 1e-6


def _transposed(w):
    return w.astype(F32).T.astype(BF)


def _kernel(x_hbm, aqkv_hbm, awo_hbm, bqkv_hbm, bwo_hbm, o_hbm,
            k_s, qt_s, vt_s, ot_s, sa_s, sb_s, kb_s,
            xb_s, aqkv_s, awo_s, bqkv_s, bwo_s,
            x_s, xn_s, pkt_s, z_s, g_s, m_s, zc_s,
            awkt_s, bwqt_s, bwvt_s, bwkt_s,
            zero_s, sem_x, sem_w, sem_o):

    def tokens(r, u=0, n=RB):
        return pl.ds(pl.multiple_of(r * RB + u * n, n), n)

    def x_copy(r):
        return pltpu.make_async_copy(x_hbm.at[tokens(r)], xb_s.at[tokens(r)], sem_x.at[r])

    def o_copy(r):
        return pltpu.make_async_copy(xb_s.at[tokens(r)], o_hbm.at[tokens(r)], sem_o.at[r])

    def a_copy(p):
        cols = slice(p * D, (p + 1) * D)
        return pltpu.make_async_copy(aqkv_hbm.at[:, cols], aqkv_s.at[:, cols], sem_w.at[p])

    late_copies = (
        a_copy(2),
        pltpu.make_async_copy(awo_hbm, awo_s, sem_w.at[3]),
        a_copy(0),
        pltpu.make_async_copy(bqkv_hbm, bqkv_s, sem_w.at[4]),
        pltpu.make_async_copy(bwo_hbm, bwo_s, sem_w.at[5]),
    )

    def phi_kt(blk, xn):
        pkt = _phi(_dot(awkt_s[...], xn, _NT))
        pkt_s[:, blk] = pkt.astype(BF)
        zp = pkt[:, 0:128]
        for t in range(1, pkt.shape[1] // 128):
            zp = zp + pkt[:, t * 128:(t + 1) * 128]
        return zp

    def lin_keys_first(r, c):
        x_copy(r).wait()

        @pl.when(r == 0)
        def _():
            for cp in late_copies:
                cp.start()

        zp = 0.0
        for u in range(RB // FB):
            blk = tokens(r, u, FB)
            x = xb_s[blk, :].astype(F32)
            x_s[blk, :] = x
            xn = _layernorm(x).astype(BF)
            xn_s[blk, :] = xn
            zp = zp + phi_kt(blk, xn)
        z_s[r] = zp
        return c

    def lin_gram(i, c):
        rt = pl.ds(pl.multiple_of(i * 128, 128), 128)
        g_s[rt, :] = _dot(pkt_s[rt, :], xn_s[...]).astype(BF)
        for p, wt_s in enumerate((bwqt_s, bwkt_s, bwvt_s)):
            cols = pl.ds(pl.multiple_of(p * D + i * 128, 128), 128)
            wt_s[rt, :] = _transposed(bqkv_s[:, cols])
        return c

    def lin_state():
        nt = D // 128
        ri = _iota((128, 128), 0)
        ci = _iota((1, 128), 1)
        kvs = []
        for i in range(nt):
            lo, hi = max(i - 1, 0), min(i + 2, nt)
            kv = _dot(g_s[i * 128:(i + 1) * 128, :], aqkv_s[:, 2 * D + lo * 128:2 * D + hi * 128])
            parts = []
            for j in range(lo, hi):
                h0 = ((ci + j * 128) // DH) * DH - i * 128
                parts.append(jnp.where((ri >= h0) & (ri < h0 + DH),
                                       kv[:, (j - lo) * 128:(j - lo + 1) * 128], 0.0))
            kvs.append((lo, hi, jnp.concatenate(parts, axis=1).astype(BF)))
        zp = z_s[0]
        for r in range(1, NRB):
            zp = zp + z_s[r]
        z = jnp.sum(zp.T, axis=0, keepdims=True)
        cd = _iota((H, D), 1)
        hd = _iota((H, D), 0) * DH
        zc_s[...] = jnp.where((cd >= hd) & (cd < hd + DH), z, 0.0).astype(BF)
        for i, (lo, hi, kv) in enumerate(kvs):
            m_s[i * 128:(i + 1) * 128, :] = _dot(kv, awo_s[lo * 128:hi * 128, :]).astype(BF)

    def lin_out_mha_proj(r, c):
        lane = _iota((FB, 128), 1)
        pq, rcp, xs, xn = {}, {}, {}, {}

        def q(u):
            pq[u] = _phi(_dot(xn_s[tokens(r, u, FB), :], aqkv_s[:, 0:D])).astype(BF)

        def den(u):
            rt = 1.0 / (_dot(zc_s[...], pq[u], _NT) + 1e-6)
            rcp[u] = jnp.concatenate([rt, jnp.zeros((128 - H, FB), F32)], axis=0).T

        def out(u):
            rb = jnp.concatenate(
                [jnp.take_along_axis(rcp[u], (lane + j * 128) // DH, axis=1) for j in range(D // 128)],
                axis=1)
            pqn = (pq[u].astype(F32) * rb).astype(BF)
            xs[u] = x_s[tokens(r, u, FB), :] + _dot(pqn, m_s[...])
            x_s[tokens(r, u, FB), :] = xs[u]

        def key(u):
            xn[u] = _layernorm(xs[u]).astype(BF)
            kt = _dot(bwkt_s[...], xn[u], _NT)
            packed = pl.ds(pl.multiple_of((r * RB + u * FB) // 2, FB // 2), FB // 2)
            for g in range(NG):
                win = kt[g * GW:min(g * GW + 128, D)]
                if win.shape[0] < 128:
                    win = jnp.concatenate([win, jnp.zeros((128 - win.shape[0], FB), F32)], axis=0)
                k = win.T.astype(BF)
                k_s[g, packed, :] = pltpu.bitcast(k, U32)
                if u % 2 == 0:
                    kv = k[CK - 16:CK, :].astype(F32)
                    for hd in range(6 * g, min(6 * g + 6, H)):
                        for d in range(DH):
                            l0 = (hd % 6) * DH + d
                            kb_s[hd, 2 * r + u // 2, d] = jnp.broadcast_to(kv[:, l0:l0 + 1], (16, 128))

        def qv(h):
            xh = jnp.concatenate([xn[2 * h], xn[2 * h + 1]], axis=0)
            qt = _dot(bwqt_s[...], xh, _NT) * Q_SCALE
            qt_s[r, 0:D, h * HB:(h + 1) * HB] = qt.astype(BF).astype(F32)
            vt_s[:, tokens(r, h, HB)] = _dot(bwvt_s[...], xh, _NT)

        for stage, u in ((q, 0), (q, 1), (den, 0), (q, 2), (den, 1), (q, 3), (out, 0), (den, 2),
                         (den, 3), (out, 1), (out, 2), (key, 0), (out, 3), (key, 1), (key, 2),
                         (qv, 0), (key, 3), (qv, 1)):
            stage(u)
        return c

    sbuf = (sa_s, sb_s)

    def load_q(g, off, qb):
        ri = _iota((128, QB), 0)
        q = qt_s[qb, pl.ds(pl.multiple_of(GW * g, 8), 128), :]
        return jnp.where((ri >= off) & (ri < off + DH), q, 0.0).astype(BF)

    def running_max(m, s):
        sm = jnp.max(s.reshape(s.shape[0] // 8, 8, QB), axis=0)
        return sm if m is None else jnp.maximum(m, sm)

    def scores_mxu(g, q, c, s_out, m):
        lo, hi = c * CK, (c + 1) * CK - (16 if c in VPU_CHUNKS else 0)
        s = _dot(pltpu.bitcast(k_s[g, lo // 2:hi // 2, :], BF), q)
        s_out[lo:hi, :] = s
        return running_max(m, s)

    def scores_vpu(h, e, t, row0, qb, s_out, m):
        qh = qt_s.at[qb, pl.ds(pl.multiple_of(row0 + zero_s[t], 8), 24)]
        c = VPU_CHUNKS[t // 2]
        acc = [None] * (QB // 128)
        for d in range(DH):
            kd = kb_s[h, c // 2, d, (t % 2) * 8:(t % 2 + 1) * 8, :]
            for n in range(QB // 128):
                qd = qh[4 * e + d:4 * e + d + 1, n * 128:(n + 1) * 128]
                pr = jnp.broadcast_to(qd, (8, 128)) * kd
                acc[n] = pr if d == 0 else acc[n] + pr
        s = jnp.concatenate(acc, axis=1)
        t0 = (c + 1) * CK - 16 + 8 * (t % 2)
        s_out[t0:t0 + 8, :] = s
        return running_max(m, s)

    def ones_row(e):
        return DH if e == 0 else 0

    def exp_pv(row0, e, c, s_in, m, acc):
        keys = slice(c * CK, (c + 1) * CK)
        p = jnp.exp2(s_in[keys, :].reshape(CK // 8, 8, QB) - m[None])
        v = jnp.where(_iota((24, CK), 0) == ones_row(e), 1.0,
                      vt_s[pl.ds(pl.multiple_of(row0, 8), 24), keys])
        o = _dot(v, p.reshape(CK, QB))
        return o if acc is None else acc + o

    def store_o(e, r0, qb, acc):
        one = ones_row(e)
        o = acc / acc[one:one + 1]
        cols = slice(qb * QB, (qb + 1) * QB)
        if e == 1:
            mid = ot_s[pl.ds(pl.multiple_of(r0 + 16, 8), 8), cols]
            o = jnp.concatenate([jnp.where(_iota((8, QB), 0) < 4, mid, o[0:8]), o[8:24]], axis=0)
        ot_s[pl.ds(pl.multiple_of(r0 + 16 * e, 8), 24), cols] = o

    def mha_pair(j, m_prev):
        r0 = 2 * DH * j
        nb = 2 * NQ
        a_ops = [(n, c) for n in range(nb) for c in range(NC)]
        b_ops = [(n - 1, c) for n, c in a_ops]
        v_prev = jnp.maximum(r0 - 2 * DH, 0)
        o_prev = jnp.where(j == 0, D, r0 - 2 * DH)
        row_max = {-1: m_prev}
        run_max, qs, accs = {}, {}, {}

        def score_step():
            n, c = a_ops.pop(0)
            e, qb = n % 2, n // 2
            if c == 0:
                qs[n] = load_q(j // 3, (j % 3) * 2 * DH + DH * e, qb)
            m = scores_mxu(j // 3, qs[n], c, sbuf[e], run_max.get(n))
            for t in range(min(c * VPU_TILES // VPU_SPREAD, VPU_TILES),
                           min((c + 1) * VPU_TILES // VPU_SPREAD, VPU_TILES)):
                m = scores_vpu(2 * j + e, e, t, r0 + 16 * e, qb, sbuf[e], m)
            run_max[n] = m
            if c == NC - 1:
                row_max[n] = jnp.broadcast_to(jnp.max(m, axis=0, keepdims=True), (8, QB))

        def pv_step():
            n, c = b_ops.pop(0)
            e, qb = n % 2, (n % nb) // 2
            rv = v_prev if n < 0 else r0
            accs[n] = exp_pv(rv + 16 * e, e, c, sbuf[e], row_max[n], accs.get(n))
            if c == NC - 1:
                store_o(e, o_prev if n < 0 else r0, qb, accs[n])

        score_step()
        while b_ops:
            if a_ops:
                score_step()
            pv_step()
        return row_max[nb - 1]

    def mha():
        m_last = lax.fori_loop(0, H // 2, mha_pair, jnp.zeros((8, QB), F32))
        acc = None
        for c in range(NC):
            acc = exp_pv(D - 24, 1, c, sb_s, m_last, acc)
        store_o(1, D - 2 * DH, NQ - 1, acc)

    def mha_out(r, h):
        ot = ot_s[0:D, tokens(r, h, HB)].astype(BF)
        return x_s[tokens(r, h, HB), :] + _dot(ot, bwo_s[...], _TN)

    def mha_out_lin_keys(r, c):
        xs = [mha_out(r, h) for h in range(2)]
        zp = 0.0
        for h in range(2):
            blk = tokens(r, h, HB)
            x_s[blk, :] = xs[h]
            xn = _layernorm(xs[h]).astype(BF)
            xn_s[blk, :] = xn
            zp = zp + phi_kt(blk, xn)
        z_s[r] = zp
        return c

    def mha_out_final(r, c):
        for h in range(2):
            xb_s[tokens(r, h, HB), :] = mha_out(r, h).astype(BF)
        o_copy(r).start()
        return c

    def layer_pair(i, c):
        lax.fori_loop(0, D // 128, lin_gram, 0)
        lin_state()
        lax.fori_loop(0, NRB, lin_out_mha_proj, 0)
        mha()

        @pl.when(i == 0)
        def _():
            lax.fori_loop(0, NRB, mha_out_lin_keys, 0)

        @pl.when(i == 1)
        def _():
            lax.fori_loop(0, NRB, mha_out_final, 0)

        return c

    x_copy(0).start()
    a_copy(1).start()
    qt_s[:, D:, :] = jnp.zeros((NQ, QROWS - D, QB), F32)
    for t in range(VPU_TILES):
        zero_s[t] = 0
    sb_s[...] = jnp.zeros(sb_s.shape, F32)
    ot_s[D:, :] = jnp.zeros((2 * DH, S), F32)
    a_copy(1).wait()
    for r in range(1, NRB):
        x_copy(r).start()
    awkt_s[...] = _transposed(aqkv_s[:, D:2 * D])
    lax.fori_loop(0, NRB, lin_keys_first, 0)
    for cp in late_copies:
        cp.wait()

    lax.fori_loop(0, 2, layer_pair, 0)
    for r in range(NRB):
        o_copy(r).wait()


@jax.jit
def pallas_interleave_layers__linear_attn_block__mha_block__prompt_kernel(
    A_x: jax.Array,
    A_wqkv: jax.Array,
    A_wo: jax.Array,
    B_x: jax.Array,
    B_wqkv: jax.Array,
    B_wo: jax.Array,
):
    del B_x
    scratch = [
        pltpu.VMEM((NG, S // 2, 128), U32),
        pltpu.VMEM((NQ, QROWS, QB), F32),
        pltpu.VMEM((D, S), F32),
        pltpu.VMEM((D + 2 * DH, S), F32),
        pltpu.VMEM((S, QB), F32),
        pltpu.VMEM((S, QB), F32),
        pltpu.VMEM((H, NC // 2, DH, 16, 128), F32),
        pltpu.VMEM((S, D), BF),
        pltpu.VMEM((D, 3 * D), BF),
        pltpu.VMEM((D, D), BF),
        pltpu.VMEM((D, 3 * D), BF),
        pltpu.VMEM((D, D), BF),
        pltpu.VMEM((S, D), F32),
        pltpu.VMEM((S, D), BF),
        pltpu.VMEM((D, S), BF),
        pltpu.VMEM((NRB, D, 128), F32),
        pltpu.VMEM((D, D), BF),
        pltpu.VMEM((D, D), BF),
        pltpu.VMEM((H, D), BF),
        pltpu.VMEM((D, D), BF),
        pltpu.VMEM((D, D), BF),
        pltpu.VMEM((D, D), BF),
        pltpu.VMEM((D, D), BF),
        pltpu.SMEM((VPU_TILES,), jnp.int32),
        pltpu.SemaphoreType.DMA((NRB,)),
        pltpu.SemaphoreType.DMA((6,)),
        pltpu.SemaphoreType.DMA((NRB,)),
    ]
    hbm = pl.BlockSpec(memory_space=pl.ANY)
    out = pl.pallas_call(
        _kernel,
        out_shape=jax.ShapeDtypeStruct((S, D), A_x.dtype),
        in_specs=[hbm] * 5,
        out_specs=hbm,
        scratch_shapes=scratch,
        compiler_params=pltpu.CompilerParams(vmem_limit_bytes=120 * 1024 * 1024),
        name="interleaved_attention",
    )(A_x.reshape(S, D), A_wqkv, A_wo, B_wqkv, B_wo)
    return out.reshape(A_x.shape)
```
